```python
import os as _os
_os.environ.setdefault("JAX_PLATFORMS", "cpu")
import jax
import jax.numpy as jnp

def _softmax(x, axis=-1):
    return jax.nn.softmax(x, axis=axis)
def _gelu(x):
    return jax.nn.gelu(x, approximate=True)
def _silu(x):
    return jax.nn.silu(x)
def _sigmoid(x):
    return jax.nn.sigmoid(x)
def _layernorm(x, axis=-1, eps=1e-5):
    m = jnp.mean(x, axis=axis, keepdims=True)
    v = jnp.var(x, axis=axis, keepdims=True)
    return (x - m) / jnp.sqrt(v + eps)
def _scatter_add(tgt, idx, src, axis=0):
    return tgt.at[idx].add(src)
def _segment_sum(src, seg, n):
    return jax.ops.segment_sum(src, seg, n)
class _Rng:
    def __init__(self, key):
        self._k = key
    def _next(self):
        self._k, sub = jax.random.split(self._k)
        return sub
    def normal(self, shape):
        return jax.random.normal(self._next(), shape, dtype=jnp.bfloat16)
    def randint(self, lo, hi, shape):
        return jax.random.randint(self._next(), shape, lo, hi, dtype=jnp.int32)
    def uniform(self, shape, lo=0.0, hi=1.0):
        return jax.random.uniform(self._next(), shape, jnp.bfloat16, lo, hi)
    def permutation(self, n):
        return jax.random.permutation(self._next(), n)


kernel_name = 'standalone__gqa_softmax__near_ridge'

def setup_inputs():
    _rng = _Rng(jax.random.key(int.from_bytes(__import__("os").urandom(4), "little")))
    _w = (lambda a: (lambda t: t.astype(jnp.bfloat16) if jnp.issubdtype(t.dtype, jnp.floating) else t)(jnp.asarray(a)))
    B, Hq, Hkv, Sq, Sk, D = 8, 16, 8, 160, 2048, 256
    return {
        "q": _w((lambda *s: _rng.normal(s) * 0.05)(B, Hq, Sq, D)),
        "k": _w((lambda *s: _rng.normal(s) * 3.2)(B, Hkv, Sk, D)),
        "v": _w((lambda *s: _rng.normal(s) * 0.05)(B, Hkv, Sk, D)),
    }

def reference(q, k, v):
    B, Hq, Sq, D = q.shape
    Hkv = k.shape[1]
    rep = Hq // Hkv
    k = jnp.repeat(k, rep, axis=1)
    v = jnp.repeat(v, rep, axis=1)
    scale = D ** -0.5
    scores = jnp.einsum("bhqd,bhkd->bhqk", q, k) * scale
    p = _softmax(scores, axis=-1)
    return jnp.einsum("bhqk,bhkd->bhqd", p, v)
```

```python
import functools

import jax
import jax.numpy as jnp
import jax.experimental.pallas as pl
import jax.experimental.pallas.tpu as pltpu


def _attn_kernel(q_ref, k_ref, v_ref, o_ref, *, scale):
    q = q_ref[0, 0]
    k = k_ref[0, 0]
    v = v_ref[0, 0]
    s = jax.lax.dot_general(
        q, k, (((1,), (1,)), ((), ())), preferred_element_type=jnp.float32
    )
    s = s * scale
    m = jnp.max(s, axis=-1, keepdims=True)
    p = jnp.exp(s - m)
    l = jnp.sum(p, axis=-1, keepdims=True)
    o = jnp.dot(p.astype(jnp.bfloat16), v, preferred_element_type=jnp.float32)
    o_ref[0, 0] = (o / l).astype(o_ref.dtype)


@jax.jit
def pallas_standalone__gqa_softmax__near_ridge_kernel(
    q: jax.Array,
    k: jax.Array,
    v: jax.Array,
):
    B, Hq, Sq, D = q.shape
    _, Hkv, Sk, _ = k.shape
    rep = Hq // Hkv
    M = rep * Sq
    qr = q.reshape(B, Hkv, M, D)
    scale = float(D) ** -0.5

    out = pl.pallas_call(
        functools.partial(_attn_kernel, scale=scale),
        grid=(B, Hkv),
        in_specs=[
            pl.BlockSpec((1, 1, M, D), lambda b, h: (b, h, 0, 0)),
            pl.BlockSpec((1, 1, Sk, D), lambda b, h: (b, h, 0, 0)),
            pl.BlockSpec((1, 1, Sk, D), lambda b, h: (b, h, 0, 0)),
        ],
        out_specs=pl.BlockSpec((1, 1, M, D), lambda b, h: (b, h, 0, 0)),
        out_shape=jax.ShapeDtypeStruct((B, Hkv, M, D), q.dtype),
        compiler_params=pltpu.CompilerParams(
            dimension_semantics=("parallel", "parallel"),
            vmem_limit_bytes=64 * 1024 * 1024,
        ),
    )(qr, k, v)
    return out.reshape(B, Hq, Sq, D)
```

```python
import functools
import math

import jax
import jax.numpy as jnp
from jax import lax
import jax.experimental.pallas as pl
import jax.experimental.pallas.tpu as pltpu

LANES = 128
SUBLANES = 8
CM = 80
KC = 8
DEP = 2
LAG = 2
NB = 16
PHASES = ((1, 6), (2, 5), (4, 12))
OUT_G = 48


def _bits(x):
    return lax.bitcast_convert_type(x, jnp.int32)


def _fold_rows(x):
    a = x[0:SUBLANES]
    for r in range(1, x.shape[0] // SUBLANES):
        a = a | x[SUBLANES * r:SUBLANES * (r + 1)]
    return a


def _after(m, zeros8):
    rep = jnp.concatenate([zeros8] * (m.shape[0] // SUBLANES), axis=0)
    return lax.bitcast_convert_type(_bits(m) | rep, jnp.float32)


def _attn_kernel(q_hbm, k_hbm, v_hbm, o_hbm, buf, obuf, in_sem, out_sem, *, scale, G):
    M = q_hbm.shape[1]
    Sk = k_hbm.shape[1]
    nch = M // CM
    ck = Sk // KC
    c = scale * math.log2(math.e)
    k_off, v_off, q_off = 0, Sk, 2 * Sk

    step = pl.program_id(0)
    nsteps = pl.num_programs(0)
    zero = lax.shift_right_logical(step, 24)

    def first_head_of(s):
        res, s0, gb = None, 0, 0
        for hs, n in PHASES:
            val = gb + hs * (s - s0)
            res = val if res is None else jnp.where(s >= s0, val, res)
            s0 += n
            gb += hs * n
        return res

    def step_of(g):
        res, s0, gb = None, 0, 0
        for hs, n in PHASES:
            if isinstance(g, int):
                if g >= gb:
                    res = s0 + (g - gb) // hs
            else:
                val = s0 + lax.div(jnp.maximum(g - gb, 0), hs)
                res = val if res is None else jnp.where(g >= gb, val, res)
            s0 += n
            gb += hs * n
        return res

    g0 = first_head_of(step)
    gprev = first_head_of(jnp.maximum(step - 1, 0))

    def in_copies(g):
        if isinstance(g, int):
            slot, si = g % NB, step_of(g) % NB
        else:
            slot, si = lax.rem(g, NB), lax.rem(step_of(g), NB)
        sem = in_sem.at[si]
        return (
            pltpu.make_async_copy(q_hbm.at[g], buf.at[slot, pl.ds(q_off, M)], sem),
            pltpu.make_async_copy(k_hbm.at[g], buf.at[slot, pl.ds(k_off, Sk)], sem),
            pltpu.make_async_copy(v_hbm.at[g], buf.at[slot, pl.ds(v_off, Sk)], sem),
        )

    big_out = pltpu.make_async_copy(
        obuf.at[pl.ds(0, OUT_G)], o_hbm.at[pl.ds(0, OUT_G)], out_sem.at[1])

    @pl.when(step == 0)
    def _():
        for g in range(NB):
            for cp in in_copies(g):
                cp.start()

    def run(H, g_lo, g_hi):
        late = g_hi > OUT_G
        has_big = g_lo <= OUT_G < g_hi
        last_phase = g_hi == G
        slot0 = lax.rem(g0, NB)
        grp = buf.at[pl.ds(slot0, H)]
        pltpu.make_async_copy(grp, grp, in_sem.at[lax.rem(step, NB)]).wait()

        def prefetch(idx):
            g = g0 + NB - H + idx

            @pl.when(jnp.logical_and(g < G, g >= gprev + NB))
            def _():
                for cp in in_copies(g):
                    cp.start()

        tasks = [(h, i * CM) for h in range(H) for i in range(nch)]
        nt = len(tasks)

        def qk(t):
            h, a = t
            q = buf[slot0 + h, pl.ds(q_off + a, CM), :]
            kk = buf[slot0 + h, pl.ds(k_off, Sk), :]
            return lax.dot_general(q, kk, (((1,), (1,)), ((), ())),
                                   preferred_element_type=jnp.float32)

        s_next = qk(tasks[0])
        ls = []
        for n, (h, a0) in enumerate(tasks):
            s = s_next
            if n + 1 < nt:
                s_next = qk(tasks[n + 1])
            if a0 == 0:
                prefetch(h)
            if has_big and n == nt - 2:
                @pl.when(g0 == OUT_G)
                def _():
                    big_out.start()

            m = jnp.max(s, axis=-1, keepdims=True)
            if n >= DEP:
                m = _after(m, _fold_rows(_bits(ls[n - DEP]) & zero))
            o = None
            l = None
            pjs = []
            for j in range(KC):
                mj = m
                if n == nt - 1 and j >= LAG:
                    pz = _bits(pjs[j - LAG]) & zero
                    a = pz[:, 0:LANES]
                    for t in range(1, ck // LANES):
                        a = a | pz[:, t * LANES:(t + 1) * LANES]
                    mj = _after(m, _fold_rows(a)[:, 0:1])
                pj = jnp.exp2((s[:, j * ck:(j + 1) * ck] - mj) * c)
                pjs.append(pj)
                for t in range(ck // LANES):
                    pt = pj[:, t * LANES:(t + 1) * LANES]
                    l = pt if l is None else l + pt
                oj = jnp.dot(pj.astype(jnp.bfloat16),
                             buf[slot0 + h, pl.ds(v_off + j * ck, ck), :],
                             preferred_element_type=jnp.float32)
                o = oj if o is None else o + oj
            l = jnp.sum(l, axis=-1, keepdims=True)
            ls.append(l)
            obuf[g0 + h, a0:a0 + CM, :] = (o / l).astype(obuf.dtype)
            if late:
                @pl.when(g0 >= OUT_G)
                def _():
                    pltpu.make_async_copy(obuf.at[g0 + h, pl.ds(a0, CM)],
                                          o_hbm.at[g0 + h, pl.ds(a0, CM)],
                                          out_sem.at[0]).start()

        if last_phase:
            @pl.when(step == nsteps - 1)
            def _():
                big_out.wait()
                pltpu.make_async_copy(obuf.at[pl.ds(OUT_G, G - OUT_G)],
                                      o_hbm.at[pl.ds(OUT_G, G - OUT_G)],
                                      out_sem.at[0]).wait()

    s0, gb = 0, 0
    for hs, n in PHASES:
        @pl.when(jnp.logical_and(step >= s0, step < s0 + n))
        def _(hs=hs, gb=gb, n=n):
            run(hs, gb, gb + hs * n)
        s0 += n
        gb += hs * n


@jax.jit
def pallas_standalone__gqa_softmax__near_ridge_kernel(
    q: jax.Array,
    k: jax.Array,
    v: jax.Array,
):
    B, Hq, Sq, D = q.shape
    _, Hkv, Sk, _ = k.shape
    rep = Hq // Hkv
    M = rep * Sq
    G = B * Hkv
    assert sum(a * b for a, b in PHASES) == G and M % CM == 0 and Sk % (KC * LANES) == 0
    gb = 0
    for hs, n in PHASES:
        assert gb % hs == 0 and NB % hs == 0
        gb += hs * n
    assert OUT_G % PHASES[-1][0] == 0 and G - PHASES[-1][0] * PHASES[-1][1] <= OUT_G < G

    qr = q.reshape(G, M, D)
    kr = k.reshape(G, Sk, D)
    vr = v.reshape(G, Sk, D)
    scale = float(D) ** -0.5
    nsteps = sum(n for _, n in PHASES)

    out = pl.pallas_call(
        functools.partial(_attn_kernel, scale=scale, G=G),
        grid=(nsteps,),
        in_specs=[pl.BlockSpec(memory_space=pl.ANY)] * 3,
        out_specs=pl.BlockSpec(memory_space=pl.ANY),
        out_shape=jax.ShapeDtypeStruct((G, M, D), q.dtype),
        scratch_shapes=[
            pltpu.VMEM((NB, 2 * Sk + M, D), q.dtype),
            pltpu.VMEM((G, M, D), q.dtype),
            pltpu.SemaphoreType.DMA((NB,)),
            pltpu.SemaphoreType.DMA((2,)),
        ],
        compiler_params=pltpu.CompilerParams(
            dimension_semantics=("arbitrary",),
            vmem_limit_bytes=110 * 1024 * 1024,
            disable_bounds_checks=True,
        ),
    )(qr, kr, vr)
    return out.reshape(B, Hq, Sq, D)
```

```python
import functools
import math

import jax
import jax.numpy as jnp
from jax import lax
import jax.experimental.pallas as pl
import jax.experimental.pallas.tpu as pltpu

LANES = 128
SUBLANES = 8
CM = 80
KC = 8
DEP = 2
LAG = 2
NB = 16
PHASES = ((1, 1), (1, 5), (2, 7), (4, 11))
OUT_G = 48


def _bits(x):
    return lax.bitcast_convert_type(x, jnp.int32)


def _fold_rows(x):
    a = x[0:SUBLANES]
    for r in range(1, x.shape[0] // SUBLANES):
        a = a | x[SUBLANES * r:SUBLANES * (r + 1)]
    return a


def _after(m, zeros8):
    rep = jnp.concatenate([zeros8] * (m.shape[0] // SUBLANES), axis=0)
    return lax.bitcast_convert_type(_bits(m) | rep, jnp.float32)


def _attn_kernel(q_hbm, k_hbm, v_hbm, o_hbm, buf, obuf, in_sem, aux_sem, *, scale, G):
    M = q_hbm.shape[1]
    Sk = k_hbm.shape[1]
    nch = M // CM
    ck = Sk // KC
    c = scale * math.log2(math.e)
    q_off, k_off, v_off = 0, M, M + Sk

    step = pl.program_id(0)
    nsteps = pl.num_programs(0)
    zero = lax.shift_right_logical(step, 24)

    def first_head_of(s):
        res, s0, gb = None, 0, 0
        for hs, n in PHASES:
            val = gb + hs * (s - s0)
            res = val if res is None else jnp.where(s >= s0, val, res)
            s0 += n
            gb += hs * n
        return res

    def step_of(g):
        res, s0, gb = None, 0, 0
        for hs, n in PHASES:
            if isinstance(g, int):
                if g >= gb:
                    res = s0 + (g - gb) // hs
            else:
                val = s0 + lax.shift_right_logical(jnp.maximum(g - gb, 0), hs.bit_length() - 1)
                res = val if res is None else jnp.where(g >= gb, val, res)
            s0 += n
            gb += hs * n
        return res

    g0 = first_head_of(step)
    gprev = first_head_of(jnp.maximum(step - 1, 0))

    def in_copies(g):
        if isinstance(g, int):
            slot, si = g % NB, step_of(g) % NB
        else:
            slot, si = g & (NB - 1), step_of(g) & (NB - 1)
        sem = in_sem.at[si]
        vsem = aux_sem.at[2] if (isinstance(g, int) and g == 0) else sem
        return (
            pltpu.make_async_copy(q_hbm.at[g], buf.at[slot, pl.ds(q_off, M)], sem),
            pltpu.make_async_copy(k_hbm.at[g], buf.at[slot, pl.ds(k_off, Sk)], sem),
            pltpu.make_async_copy(v_hbm.at[g], buf.at[slot, pl.ds(v_off, Sk)], vsem),
        )

    big_out = pltpu.make_async_copy(
        obuf.at[pl.ds(0, OUT_G)], o_hbm.at[pl.ds(0, OUT_G)], aux_sem.at[1])

    def run(H, g_lo, g_hi):
        head0 = g_hi == 1
        if head0:
            for g in range(NB):
                for cp in in_copies(g):
                    cp.start()

        late = g_hi > OUT_G
        has_big = g_lo <= OUT_G < g_hi
        last_phase = g_hi == G
        slot0 = g0 & (NB - 1)
        if head0:
            grp = buf.at[0, pl.ds(q_off, M + Sk)]
            pltpu.make_async_copy(grp, grp, in_sem.at[0]).wait()
        else:
            grp = buf.at[pl.ds(slot0, H)]
            pltpu.make_async_copy(grp, grp, in_sem.at[step & (NB - 1)]).wait()

        def prefetch(idx):
            g = g0 + NB - H + idx

            @pl.when(jnp.logical_and(g < G, g >= gprev + NB))
            def _():
                for cp in in_copies(g):
                    cp.start()

        tasks = [(h, i * CM) for h in range(H) for i in range(nch)]
        nt = len(tasks)

        def qk(t):
            h, a = t
            q = buf[slot0 + h, pl.ds(q_off + a, CM), :]
            kk = buf[slot0 + h, pl.ds(k_off, Sk), :]
            return lax.dot_general(q, kk, (((1,), (1,)), ((), ())),
                                   preferred_element_type=jnp.float32)

        if head0:
            s_all = [qk(t) for t in tasks]
        else:
            s_next = qk(tasks[0])
        ls = []
        for n, (h, a0) in enumerate(tasks):
            if head0:
                s = s_all[n]
                if n == 0:
                    grp = buf.at[0, pl.ds(v_off, Sk)]
                    pltpu.make_async_copy(grp, grp, aux_sem.at[2]).wait()
            else:
                s = s_next
                if n + 1 < nt:
                    s_next = qk(tasks[n + 1])
                if a0 == 0:
                    prefetch(h)
            if has_big and n == nt - 2:
                @pl.when(g0 == OUT_G)
                def _():
                    big_out.start()

            m = jnp.max(s, axis=-1, keepdims=True)
            if n >= DEP:
                m = _after(m, _fold_rows(_bits(ls[n - DEP]) & zero))
            o = None
            l = None
            pjs = []
            for j in range(KC):
                mj = m
                if n == nt - 1 and j >= LAG:
                    pz = _bits(pjs[j - LAG]) & zero
                    a = pz[:, 0:LANES]
                    for t in range(1, ck // LANES):
                        a = a | pz[:, t * LANES:(t + 1) * LANES]
                    mj = _after(m, _fold_rows(a)[:, 0:1])
                pj = jnp.exp2((s[:, j * ck:(j + 1) * ck] - mj) * c)
                pjs.append(pj)
                for t in range(ck // LANES):
                    pt = pj[:, t * LANES:(t + 1) * LANES]
                    l = pt if l is None else l + pt
                oj = jnp.dot(pj.astype(jnp.bfloat16),
                             buf[slot0 + h, pl.ds(v_off + j * ck, ck), :],
                             preferred_element_type=jnp.float32)
                o = oj if o is None else o + oj
            l = jnp.sum(l, axis=-1, keepdims=True)
            ls.append(l)
            obuf[g0 + h, a0:a0 + CM, :] = (o / l).astype(obuf.dtype)
            if late:
                @pl.when(g0 >= OUT_G)
                def _():
                    pltpu.make_async_copy(obuf.at[g0 + h, pl.ds(a0, CM)],
                                          o_hbm.at[g0 + h, pl.ds(a0, CM)],
                                          aux_sem.at[0]).start()

        if last_phase:
            @pl.when(step == nsteps - 1)
            def _():
                big_out.wait()
                pltpu.make_async_copy(obuf.at[pl.ds(OUT_G, G - OUT_G)],
                                      o_hbm.at[pl.ds(OUT_G, G - OUT_G)],
                                      aux_sem.at[0]).wait()

    bounds, s0, gb = [], 0, 0
    for hs, n in PHASES:
        bounds.append((s0, hs, gb, gb + hs * n))
        s0 += n
        gb += hs * n

    def dispatch(i):
        s_lo, hs, g_lo, g_hi = bounds[i]
        if i == 0:
            run(hs, g_lo, g_hi)
        else:
            lax.cond(step >= s_lo, lambda: run(hs, g_lo, g_hi), lambda: dispatch(i - 1))

    dispatch(len(bounds) - 1)


@jax.jit
def pallas_standalone__gqa_softmax__near_ridge_kernel(
    q: jax.Array,
    k: jax.Array,
    v: jax.Array,
):
    B, Hq, Sq, D = q.shape
    _, Hkv, Sk, _ = k.shape
    rep = Hq // Hkv
    M = rep * Sq
    G = B * Hkv
    assert sum(a * b for a, b in PHASES) == G and M % CM == 0 and Sk % (KC * LANES) == 0
    assert NB & (NB - 1) == 0 and PHASES[0] == (1, 1)
    gb = 0
    for hs, n in PHASES:
        assert gb % hs == 0 and NB % hs == 0 and hs & (hs - 1) == 0
        gb += hs * n
    assert OUT_G % PHASES[-1][0] == 0 and G - PHASES[-1][0] * PHASES[-1][1] <= OUT_G < G

    qr = q.reshape(G, M, D)
    kr = k.reshape(G, Sk, D)
    vr = v.reshape(G, Sk, D)
    scale = float(D) ** -0.5
    nsteps = sum(n for _, n in PHASES)

    out = pl.pallas_call(
        functools.partial(_attn_kernel, scale=scale, G=G),
        grid=(nsteps,),
        in_specs=[pl.BlockSpec(memory_space=pl.ANY)] * 3,
        out_specs=pl.BlockSpec(memory_space=pl.ANY),
        out_shape=jax.ShapeDtypeStruct((G, M, D), q.dtype),
        scratch_shapes=[
            pltpu.VMEM((NB, M + 2 * Sk, D), q.dtype),
            pltpu.VMEM((G, M, D), q.dtype),
            pltpu.SemaphoreType.DMA((NB,)),
            pltpu.SemaphoreType.DMA((3,)),
        ],
        compiler_params=pltpu.CompilerParams(
            dimension_semantics=("arbitrary",),
            vmem_limit_bytes=110 * 1024 * 1024,
            disable_bounds_checks=True,
        ),
    )(qr, kr, vr)
    return out.reshape(B, Hq, Sq, D)
```
